```python
import os as _os
_os.environ.setdefault("JAX_PLATFORMS", "cpu")
import jax
import jax.numpy as jnp

def _softmax(x, axis=-1):
    return jax.nn.softmax(x, axis=axis)
def _gelu(x):
    return jax.nn.gelu(x, approximate=True)
def _silu(x):
    return jax.nn.silu(x)
def _sigmoid(x):
    return jax.nn.sigmoid(x)
def _layernorm(x, axis=-1, eps=1e-5):
    m = jnp.mean(x, axis=axis, keepdims=True)
    v = jnp.var(x, axis=axis, keepdims=True)
    return (x - m) / jnp.sqrt(v + eps)
def _scatter_add(tgt, idx, src, axis=0):
    return tgt.at[idx].add(src)
def _segment_sum(src, seg, n):
    return jax.ops.segment_sum(src, seg, n)
class _Rng:
    def __init__(self, key):
        self._k = key
    def _next(self):
        self._k, sub = jax.random.split(self._k)
        return sub
    def normal(self, shape):
        return jax.random.normal(self._next(), shape, dtype=jnp.bfloat16)
    def randint(self, lo, hi, shape):
        return jax.random.randint(self._next(), shape, lo, hi, dtype=jnp.int32)
    def uniform(self, shape, lo=0.0, hi=1.0):
        return jax.random.uniform(self._next(), shape, jnp.bfloat16, lo, hi)
    def permutation(self, n):
        return jax.random.permutation(self._next(), n)


kernel_name = 'recurrent_scan__sliding_block__dense_activation_mish__prompt'

def setup_inputs():
    _rng = _Rng(jax.random.key(int.from_bytes(__import__("os").urandom(4), "little")))
    _w = (lambda a: (lambda t: t.astype(jnp.bfloat16) if jnp.issubdtype(t.dtype, jnp.floating) else t)(jnp.asarray(a)))
    def _A_setup():
        B, S, D = 1, 2048, 576
        return {
            "x": _w((lambda *s: _rng.normal(s) * 0.05)(B, S, D)),
            "wqkv": _w((lambda *s: _rng.normal(s) * 0.1)(D, 3 * D)),
            "wo": _w((lambda *s: _rng.normal(s) * 0.1)(D, D)),
        }
    _A_in = _A_setup()

    def _B_setup():
        B, S, D, F = 1, 2048, 576, 4608
        return {
            "x": _w((lambda *s: _rng.normal(s) * 0.05)(B, S, D)),
            "w1": _w((lambda *s: _rng.normal(s) * 0.05)(D, F) * (D ** -0.5)),
            "b1": _w((lambda *s: _rng.normal(s) * 0.05)(F)),
            "w2": _w((lambda *s: _rng.normal(s) * 0.05)(F, D) * (F ** -0.5)),
        }
    _B_in = _B_setup()

    return {
        "A_x": _A_in["x"],
        "A_wqkv": _A_in["wqkv"],
        "A_wo": _A_in["wo"],
        "B_x": _B_in["x"],
        "B_w1": _B_in["w1"],
        "B_b1": _B_in["b1"],
        "B_w2": _B_in["w2"],
    }

def reference(A_x, A_wqkv, A_wo, B_x, B_w1, B_b1, B_w2):
    def _A_ref(x, wqkv, wo):
        B, S, D = x.shape
        H = 32; Dh = D // H; W = 256
        qkv = (lambda x, *d: x.transpose(*d))((x @ wqkv).reshape(B, S, 3, H, Dh), 2, 0, 3, 1, 4)
        q, k, v = qkv[0], qkv[1], qkv[2]
        scores = jnp.einsum("bhqd,bhkd->bhqk", q, k) * (Dh ** -0.5)
        idx = jnp.arange(S)
        mask = (idx[:, None] - idx[None, :] >= 0) & (idx[:, None] - idx[None, :] < W)
        scores = jnp.where(mask[None, None], scores, -1e9)
        p = _softmax(scores, axis=-1)
        o = jnp.einsum("bhqk,bhkd->bhqd", p, v)
        return (lambda x, *d: x.transpose(*d))(o, 0, 2, 1, 3).reshape(B, S, D) @ wo

    def _B_ref(x, w1, b1, w2):
        h = jnp.einsum("bsd,df->bsf", x, w1) + b1
        sp = jnp.log1p(jnp.exp(-jnp.abs(h))) + jnp.where(h > 0, h, jnp.zeros_like(h))
        act = h * jnp.tanh(sp)
        return jnp.einsum("bsf,fd->bsd", act, w2)

    x = A_x
    xn = _layernorm(x, axis=-1)
    s = _A_ref(xn, A_wqkv, A_wo)
    g = _silu(_B_ref(xn, B_w1, B_b1, B_w2))
    return x + s * g
```

```python
import jax
import jax.numpy as jnp
import jax.experimental.pallas as pl
import jax.experimental.pallas.tpu as pltpu

S, D, F, H, DH, W = 2048, 576, 4608, 32, 18, 256
HPT = 7
NT = 5
DP = NT * 128
TA = 256
TB = 256
FC = 128
NC = F // FC
DEF = 0; Y = 1
LOG2E = 1.4426950408889634
ONE2 = 0x3F803F80
NEG2 = 0xCE6ECE6E - (1 << 32)
bf16, f32, i32 = jnp.bfloat16, jnp.float32, jnp.int32
NT_DIMS = (((1,), (1,)), ((), ()))


def mo(x, n):
    return x if isinstance(x, int) else pl.multiple_of(x, n)


def _iota(shape, d):
    return jax.lax.broadcasted_iota(i32, shape, d)


def _kernel(xT_hbm, wqkv_hbm, wo_hbm, w1_hbm, b1_ref, w2T_hbm, oT_hbm,
            xT, wqk_in, wv, wo, w1, w2T, wqk, wvT, woT, xn, xnT, q_s, k_s, kc_s, vT_s,
            oT_s, yT_s, sT_s, s_s, a_s, out_s, sem_in, sem_out):
    def x_copy(i):
        lo, n = (0, 2 * TA) if i == 0 else (2 * TA, S - 2 * TA)
        return pltpu.make_async_copy(xT_hbm.at[:, pl.ds(lo, n)], xT.at[:, pl.ds(lo, n)], sem_in.at[i])
    cp_qk = pltpu.make_async_copy(wqkv_hbm.at[:, pl.ds(0, 2 * D)], wqk_in, sem_in.at[2])
    cp_v = pltpu.make_async_copy(wqkv_hbm.at[:, pl.ds(2 * D, D)], wv, sem_in.at[3])
    cp_wo = pltpu.make_async_copy(wo_hbm, wo, sem_in.at[4])
    cp_w1 = pltpu.make_async_copy(w1_hbm, w1.at[pl.ds(0, D), :], sem_in.at[5])
    cp_w2 = pltpu.make_async_copy(w2T_hbm, w2T, sem_in.at[6])
    x_copy(0).start()
    cp_qk.start()

    k_s[pl.ds(0, W // 2), :] = jnp.zeros((W // 2, DP), i32)
    for h in range(H):
        kc_s[h, pl.ds(0, 80), :] = jnp.where(_iota((80, 128), 1) >= 124, NEG2, 0)
    vT_s[:, pl.ds(0, W)] = jnp.zeros((D, W), bf16)
    b1 = jnp.broadcast_to(b1_ref[...].astype(f32).reshape(1, F), (DP - D, F))
    w1[pl.ds(D, DP - D), :] = jnp.where(_iota((DP - D, F), 0) == 0, b1, 0.0).astype(bf16)
    yT_s[...] = jnp.zeros(yT_s.shape, f32)
    sT_s[...] = jnp.zeros(sT_s.shape, f32)
    a_s[...] = jnp.zeros(a_s.shape, bf16)
    wqk[...] = jnp.zeros(wqk.shape, bf16)

    def ln(i):
        t0 = mo(i * TA, TA)
        x = xT[:, pl.ds(t0, TA)].astype(f32)
        m = jnp.mean(x, axis=0, keepdims=True)
        xc = x - m
        v = jnp.mean(xc * xc, axis=0, keepdims=True)
        y = xc * jax.lax.rsqrt(v + 1e-5)
        ext = jnp.concatenate([y, jnp.where(_iota((DP - D, TA), 0) == 0, 1.0, 0.0)], axis=0)
        xn[pl.ds(t0, TA), :] = ext.T.astype(bf16)
        xnT[:, pl.ds(t0, TA)] = y.astype(bf16)

    def proj(i, extra):
        t0 = mo(i * TA, TA)
        qk = jnp.dot(xn[pl.ds(t0, TA), :], wqk[...], preferred_element_type=f32)
        extra()
        q_s[pl.ds(t0, TA), :] = (qk[:, :DP] * (DH ** -0.5 * LOG2E)).astype(bf16)
        k_s[pl.ds(mo((W + t0) // 2, TA // 2), TA // 2), :] = pltpu.bitcast(qk[:, DP:].astype(bf16), i32)

    x_copy(0).wait()
    cp_qk.wait()
    x_copy(1).start()
    cp_v.start()
    cp_wo.start()
    ln(0)
    for part in range(2):
        for t in range(NT):
            n = min(HPT, H - t * HPT) * DH
            wqk[pl.ds(0, D), pl.ds((part * NT + t) * 128, n)] = wqk_in[:, pl.ds(part * D + t * HPT * DH, n)]
    na = S // TA
    nxt = lambda i: jnp.where(i < na, i, 0)
    proj(0, lambda: ln(1))
    x_copy(1).wait()
    cp_v.wait()
    cp_w1.start()
    cp_w2.start()
    wvT[...] = wv[...].astype(f32).T.astype(bf16)

    def v_stair(i):
        t0 = mo(i * TA, TA)
        vT_s[:, pl.ds(W + t0, TA)] = jnp.dot(wvT[...], xnT[:, pl.ds(t0, TA)], preferred_element_type=f32).astype(bf16)
        r0 = mo(t0 // 2 + 80, 16)
        lane = _iota((TA // 2, 128), 1)
        key = 2 * (_iota((TA // 2, 128), 0) + r0) + 32 * (lane - 124)
        fill = jnp.where((lane >= 124) & (key < W), NEG2, 0)
        for t in range(NT):
            src = k_s[pl.ds(r0, TA // 2 + 48), pl.ds(t * 128, 128)]
            rolled = {0: src}
            for j in range(min(HPT, H - t * HPT)):
                x = fill
                for g in range(4):
                    if g - j not in rolled:
                        rolled[g - j] = pltpu.roll(src, (DH * (g - j)) % 128, 1)
                    x = jnp.where((lane >= g * DH) & (lane < (g + 1) * DH), rolled[g - j][16 * g:16 * g + TA // 2], x)
                kc_s[t * HPT + j, pl.ds(r0, TA // 2), :] = x

    def phase_a(i, c):
        v_stair(i - 1)
        proj(i, lambda: ln(nxt(i + 1)))
        return c
    jax.lax.fori_loop(1, na, phase_a, 0)
    cp_wo.wait()
    v_stair(na - 1)
    woT[...] = wo[...].astype(f32).T.astype(bf16)
    cp_w1.wait()
    cp_w2.wait()

    def out_copy(i, slot):
        return pltpu.make_async_copy(out_s.at[slot], oT_hbm.at[:, pl.ds(i * TB, TB)], sem_out.at[slot])

    def qk_unit(t0, qb, h):
        t, j = divmod(h, HPT)
        ln_ = _iota((16, 128), 1)
        qt = pltpu.bitcast(q_s[pl.ds(t0 + qb * 128, 128), pl.ds(t * 128, 128)], i32)
        parts = []
        for g in range(4):
            x = qt[16 * g:16 * g + 16]
            if g != j:
                x = pltpu.roll(x, (DH * (g - j)) % 128, 1)
            parts.append(jnp.where((ln_ >= g * DH) & (ln_ < (g + 1) * DH), x, jnp.where(ln_ == 124 + g, ONE2, 0)))
        qm = pltpu.bitcast(jnp.concatenate(parts, axis=0), bf16)
        kt = pltpu.bitcast(kc_s[h, pl.ds(pl.multiple_of((t0 + qb * 128) // 2, 64), 144), :], bf16)
        return jax.lax.dot_general(kt, qm, NT_DIMS, preferred_element_type=f32)

    def sm_unit(s):
        ln_ = _iota((32, 128), 1)
        up = _iota((32, 128), 0) > (ln_ & 31)
        s0 = jnp.where(up, s[0:32], s[256:288])
        s1 = s[32:256]
        mx = jnp.maximum(jnp.max(s0, axis=0, keepdims=True), jnp.max(s1, axis=0, keepdims=True))
        p0 = jnp.exp2(s0 - mx)
        p1 = jnp.exp2(s1 - mx)
        den = jnp.sum(p0, axis=0, keepdims=True) + jnp.sum(p1, axis=0, keepdims=True)
        c = [jnp.where(up, p0, 0.0)] + [p1[32 * n:32 * n + 32] for n in range(7)] + [jnp.where(up, 0.0, p0)]
        odd = (ln_ & 32) != 0
        hi = ln_ >= 64
        c = [jnp.where(odd, c[n - 1] if n >= 1 else 0.0, c[n] if n < 9 else 0.0) for n in range(10)]
        c = [jnp.where(hi, c[n - 2] if n >= 2 else 0.0, c[n] if n < 10 else 0.0) for n in range(12)]
        return jnp.concatenate(c, axis=0).astype(bf16), 1.0 / den

    def pv_unit(t0, qb, h, p, inv):
        a = (h * DH) // 16 * 16
        vt = vT_s[pl.ds(a, 32), pl.ds(t0 + qb * 128, 384)]
        o = jnp.dot(vt, p, preferred_element_type=f32) * inv
        lo, hi = h * DH, (h + 1) * DH
        for g in range(lo // 8, (hi + 7) // 8):
            blk = o[g * 8 - a:g * 8 - a + 8]
            dst = (pl.ds(g * 8, 8), pl.ds(qb * 128, 128))
            if g * 8 < lo:
                blk = jnp.where(_iota((8, 128), 0) >= lo - g * 8, blk, oT_s[dst])
            oT_s[dst] = blk

    def f1(t0, c):
        return jnp.dot(xn[pl.ds(t0, TB), :], w1[:, pl.ds(c * FC, FC)], preferred_element_type=f32)

    def mish(hh):
        e = jnp.exp2(jnp.minimum(hh, 20.0) * LOG2E)
        n = e * (e + 2.0)
        return (hh * n * pl.reciprocal(n + 2.0, approx=True)).astype(bf16)

    def f2(c, act):
        y = jax.lax.dot_general(w2T[:, pl.ds(c * FC * Y, FC * Y)], act, NT_DIMS, preferred_element_type=f32)
        if c == 0:
            yT_s[...] = y
        else:
            yT_s[...] += y

    def combine(i, slot):
        y = yT_s[...]
        g = y * (1.0 / (1.0 + jnp.exp2(y * (-LOG2E))))
        out_s[slot] = (xT[:, pl.ds(pl.multiple_of(i * TB, TB), TB)].astype(f32) + sT_s[...] * g).astype(bf16)

    def phase_b(i, c):
        t0 = pl.multiple_of(i * TB, TB)
        slot = i % 2
        nq = TB // 128

        @pl.when(i >= 3)
        def _():
            out_copy(i - 3, 1 - slot).wait()
        pv, hv, av = {}, {}, {}
        un = lambda j: [u for u in range(H * nq) if u * 32 // (H * nq) == j]
        for j in range(NC + 2 - DEF):
            if j == 0 and DEF:
                f2(NC - 1, a_s[...])
            for u in un(j):
                s_s[j % 2, u % nq] = qk_unit(t0, u % nq, u // nq)
            if j < NC:
                hv[j] = f1(t0, j)
            for u in un(j - 1):
                pv[u] = sm_unit(s_s[(j - 1) % 2, u % nq])
            if 0 <= j - 1 < NC:
                av[j - 1] = mish(hv.pop(j - 1))
            if j == 1:
                combine(jnp.maximum(i - 1, 0), 1 - slot)
            for u in un(j - 2):
                pv_unit(t0, u % nq, u // nq, *pv.pop(u))
            if 0 <= j - 2 < NC and (j - 2) % Y == Y - 1:
                f2((j - 2) // Y, jnp.concatenate([av.pop(j - 2 - Y + 1 + z) for z in range(Y)], axis=1))
            if j == 35:
                sT_s[...] = jnp.dot(woT[...], oT_s[...].astype(bf16), preferred_element_type=f32)
        if DEF:
            a_s[...] = av.pop(NC - 1)

        @pl.when(i >= 1)
        def _():
            out_copy(i - 1, 1 - slot).start()
        return c

    nb = S // TB
    jax.lax.fori_loop(0, nb, phase_b, 0)
    out_copy(nb - 3, (nb - 3) % 2).wait()
    out_copy(nb - 2, (nb - 2) % 2).wait()
    if DEF:
        f2(NC - 1, a_s[...])
    combine(nb - 1, (nb - 1) % 2)
    out_copy(nb - 1, (nb - 1) % 2).start()
    out_copy(nb - 1, (nb - 1) % 2).wait()


@jax.jit
def pallas_recurrent_scan__sliding_block__dense_activation_mish__prompt_kernel(A_x, A_wqkv, A_wo, B_x, B_w1, B_b1, B_w2):
    del B_x
    any_spec = pl.BlockSpec(memory_space=pl.ANY)
    V = pltpu.VMEM
    oT = pl.pallas_call(
        _kernel,
        out_shape=jax.ShapeDtypeStruct((D, S), bf16),
        in_specs=[any_spec, any_spec, any_spec, any_spec, pl.BlockSpec(memory_space=pltpu.VMEM), any_spec],
        out_specs=any_spec,
        scratch_shapes=[
            V((D, S), bf16), V((D, 2 * D), bf16), V((D, D), bf16), V((D, D), bf16),
            V((DP, F), bf16), V((D, F), bf16),
            V((DP, 2 * DP), bf16), V((D, D), bf16), V((D, D), bf16),
            V((S, DP), bf16), V((D, S), bf16), V((S, DP), bf16), V(((S + W) // 2, DP), i32),
            V((H, (S + W) // 2, 128), i32), V((D, S + W), bf16),
            V((D, TB), f32), V((D, TB), f32), V((D, TB), f32), V((2, TB // 128, 288, 128), f32),
            V((TB, FC), bf16), V((2, D, TB), bf16),
            pltpu.SemaphoreType.DMA((7,)), pltpu.SemaphoreType.DMA((2,)),
        ],
        compiler_params=pltpu.CompilerParams(
            vmem_limit_bytes=100 * 2**20,
            flags={"XLA_TPU_EVENLY_DISTRIBUTE_CRITICAL_NODES": True}),
        name="fused_block",
    )(A_x[0].T, A_wqkv, A_wo, B_w1, B_b1, B_w2.T)
    return oT.T[None]
```

```python
import jax
import jax.numpy as jnp
import jax.experimental.pallas as pl
import jax.experimental.pallas.tpu as pltpu

S, D, F, H, DH, W = 2048, 576, 4608, 32, 18, 256
HPT = 7
NT = 5
DP = NT * 128
TA = 256
TB = 256
FC = 128
NC = F // FC
DEF = 0; Y = 1
LOG2E = 1.4426950408889634
L_HI = 1.4453125
ONE2 = 0x3F803F80
NEG2 = 0xCE6ECE6E - (1 << 32)
bf16, f32, i32 = jnp.bfloat16, jnp.float32, jnp.int32
NT_DIMS = (((1,), (1,)), ((), ()))


def mo(x, n):
    return x if isinstance(x, int) else pl.multiple_of(x, n)


def _iota(shape, d):
    return jax.lax.broadcasted_iota(i32, shape, d)


def flag_lane(h):
    return (h % HPT + 4) % HPT * DH


def pack16(x):
    lo = jnp.concatenate([x[r:r + 8] for r in range(0, x.shape[0], 16)], axis=0)
    hi = jnp.concatenate([x[r + 8:r + 16] for r in range(0, x.shape[0], 16)], axis=0)
    return pltpu.pack_elementwise([lo, hi], packed_dtype=bf16).astype(i32)


def _kernel(xT_hbm, wqkv_hbm, wo_hbm, w1_hbm, b1_ref, w2T_hbm, oT_hbm,
            xT, wqk_in, wv, wo, w1, w2T, wqk, wvT, woT, xn, xp, xs, q_s, k_s, kc_s, vT_s,
            oT_s, yT_s, sT_s, s_s, a_s, out_s, sem_in, sem_out):
    def x_copy(i):
        lo, n = (0, 2 * TA) if i == 0 else (2 * TA, S - 2 * TA)
        return pltpu.make_async_copy(xT_hbm.at[:, pl.ds(lo, n)], xT.at[:, pl.ds(lo, n)], sem_in.at[i])
    cp_qk = pltpu.make_async_copy(wqkv_hbm.at[:, pl.ds(0, 2 * D)], wqk_in, sem_in.at[2])
    cp_v = pltpu.make_async_copy(wqkv_hbm.at[:, pl.ds(2 * D, D)], wv, sem_in.at[3])
    cp_wo = pltpu.make_async_copy(wo_hbm, wo, sem_in.at[4])
    cp_w1 = pltpu.make_async_copy(w1_hbm, w1.at[pl.ds(0, D), :], sem_in.at[5])
    cp_w2 = pltpu.make_async_copy(w2T_hbm, w2T, sem_in.at[6])
    x_copy(0).start()
    cp_qk.start()

    k_s[pl.ds(0, W // 2), :] = jnp.zeros((W // 2, DP), i32)
    for h in range(H):
        fl = _iota((80, 128), 1) - flag_lane(h)
        kc_s[h, pl.ds(0, 80), :] = jnp.where((fl >= 0) & (fl < 4), NEG2, 0)
    vT_s[:, pl.ds(0, W)] = jnp.zeros((D, W), bf16)
    b1 = jnp.broadcast_to(b1_ref[...].astype(f32).reshape(1, F), (DP - D, F))
    w1[pl.ds(D, DP - D), :] = jnp.where(_iota((DP - D, F), 0) < 2, b1, 0.0).astype(bf16)
    yT_s[...] = jnp.zeros(yT_s.shape, f32)
    sT_s[...] = jnp.zeros(sT_s.shape, f32)
    a_s[...] = jnp.zeros(a_s.shape, bf16)
    wqk[...] = jnp.zeros(wqk.shape, bf16)

    def ln(i):
        t0 = mo(i * TA, TA)
        x = xT[:, pl.ds(t0, TA)].astype(f32)
        m = jnp.mean(x, axis=0, keepdims=True)
        xc = x - m
        v = jnp.mean(xc * xc, axis=0, keepdims=True)
        y = xc * jax.lax.rsqrt(v + 1e-5)
        ext = jnp.concatenate([y, jnp.where(_iota((DP - D, TA), 0) == 0, 1.0, 0.0)], axis=0)
        et = ext.T
        xn[...] = et.astype(bf16)
        xp[pl.ds(mo(t0 // 2, TA // 2), TA // 2), :] = pack16(et)
        ll = _iota((TA, DP), 1)
        xs[pl.ds(t0, TA), :] = jnp.where(ll == D, L_HI, jnp.where(ll == D + 1, LOG2E - L_HI, et * LOG2E)).astype(bf16)

    def proj(i, extra):
        t0 = mo(i * TA, TA)
        qk = jnp.dot(xn[...], wqk[...], preferred_element_type=f32)
        extra()
        q_s[pl.ds(t0, TA), :] = (qk[:, :DP] * (DH ** -0.5 * LOG2E)).astype(bf16)
        k_s[pl.ds(mo((W + t0) // 2, TA // 2), TA // 2), :] = pltpu.bitcast(qk[:, DP:].astype(bf16), i32)

    x_copy(0).wait()
    cp_qk.wait()
    x_copy(1).start()
    cp_v.start()
    cp_wo.start()
    ln(0)
    for part in range(2):
        for t in range(NT):
            n = min(HPT, H - t * HPT) * DH
            wqk[pl.ds(0, D), pl.ds((part * NT + t) * 128, n)] = wqk_in[:, pl.ds(part * D + t * HPT * DH, n)]
    na = S // TA
    nxt = lambda i: jnp.where(i < na, i, 0)
    proj(0, lambda: ln(1))
    x_copy(1).wait()
    cp_v.wait()
    cp_w1.start()
    cp_w2.start()
    wvT[...] = wv[...].astype(f32).T.astype(bf16)

    def v_stair(i):
        t0 = mo(i * TA, TA)
        vT_s[:, pl.ds(W + t0, TA)] = jax.lax.dot_general(wvT[...], pltpu.bitcast(xp[pl.ds(mo(t0 // 2, TA // 2), TA // 2), pl.ds(0, D)], bf16), NT_DIMS, preferred_element_type=f32).astype(bf16)
        r0 = mo(t0 // 2 + 80, 16)
        lane = _iota((TA // 2, 128), 1)
        for t in range(NT):
            rolled = {}
            for j in range(min(HPT, H - t * HPT)):
                x = 0
                for g in range(4):
                    sl = (j + g) % HPT
                    if sl - j not in rolled:
                        src = k_s[pl.ds(r0 + 16 * g, TA // 2), pl.ds(t * 128, 128)]
                        rolled[sl - j] = src if g == 0 else pltpu.roll(src, (DH * (sl - j)) % 128, 1)
                    x = jnp.where((lane >= sl * DH) & (lane < (sl + 1) * DH), rolled[sl - j], x)
                kc_s[t * HPT + j, pl.ds(r0, TA // 2), :] = x

    def phase_a(i, c):
        v_stair(i - 1)
        proj(i, lambda: ln(nxt(i + 1)))
        return c
    jax.lax.fori_loop(1, na, phase_a, 0)
    cp_wo.wait()
    v_stair(na - 1)
    for h in range(H):
        fl = _iota((48, 128), 1) - flag_lane(h)
        pad = (fl >= 0) & (fl < 4) & (2 * (_iota((48, 128), 0) + 80) + 32 * fl < W)
        kc_s[h, pl.ds(80, 48), :] = jnp.where(pad, NEG2, kc_s[h, pl.ds(80, 48), :])
    woT[...] = wo[...].astype(f32).T.astype(bf16)
    cp_w1.wait()
    cp_w2.wait()

    def out_copy(i, slot):
        return pltpu.make_async_copy(out_s.at[slot], oT_hbm.at[:, pl.ds(i * TB, TB)], sem_out.at[slot])

    def qk_unit(t0, qb, h):
        t, j = divmod(h, HPT)
        ln_ = _iota((16, 128), 1)
        qt = pltpu.bitcast(q_s[pl.ds(t0 + qb * 128, 128), pl.ds(t * 128, 128)], i32)
        parts = []
        for g in range(4):
            x = qt[16 * g:16 * g + 16]
            sl = (j + g) % HPT
            if g:
                x = pltpu.roll(x, (DH * (sl - j)) % 128, 1)
            parts.append(jnp.where((ln_ >= sl * DH) & (ln_ < (sl + 1) * DH), x, jnp.where(ln_ == flag_lane(h) + g, ONE2, 0)))
        qm = pltpu.bitcast(jnp.concatenate(parts, axis=0), bf16)
        kt = pltpu.bitcast(kc_s[h, pl.ds(pl.multiple_of((t0 + qb * 128) // 2, 64), 144), :], bf16)
        return jax.lax.dot_general(kt, qm, NT_DIMS, preferred_element_type=f32)

    def sm_unit(s):
        ln_ = _iota((32, 128), 1)
        up = _iota((32, 128), 0) > (ln_ & 31)
        s0 = jnp.where(up, s[0:32], s[256:288])
        s1 = s[32:256]
        mx = jnp.maximum(jnp.max(s0, axis=0, keepdims=True), jnp.max(s1, axis=0, keepdims=True))
        p0 = jnp.exp2(s0 - mx)
        p1 = jnp.exp2(s1 - mx)
        c = [jnp.where(up, p0, 0.0)] + [p1[32 * n:32 * n + 32] for n in range(7)] + [jnp.where(up, 0.0, p0)]
        c = [pack16(x) for x in c]
        l16 = _iota((16, 128), 1)
        odd = (l16 & 32) != 0
        hi = l16 >= 64
        c = [jnp.where(odd, c[n - 1] if n >= 1 else 0, c[n] if n < 9 else 0) for n in range(10)]
        c = [jnp.where(hi, c[n - 2] if n >= 2 else 0, c[n] if n < 10 else 0) for n in range(12)]
        return pltpu.bitcast(jnp.concatenate(c, axis=0), bf16)

    def pv_unit(t0, qb, h, p):
        a = (h * DH) // 16 * 16
        vt = vT_s[pl.ds(a, 32), pl.ds(t0 + qb * 128, 384)]
        lo, hi = h * DH, (h + 1) * DH
        r = 0 if lo > a else 30
        vt = pltpu.bitcast(jnp.where(_iota((16, 384), 0) == r // 2, ONE2, pltpu.bitcast(vt, i32)), bf16)
        o = jnp.dot(vt, p, preferred_element_type=f32)
        o = o * (1.0 / o[r:r + 1])
        for g in range(lo // 8, (hi + 7) // 8):
            blk = o[g * 8 - a:g * 8 - a + 8]
            dst = (pl.ds(g * 8, 8), pl.ds(qb * 128, 128))
            if g * 8 < lo:
                blk = jnp.where(_iota((8, 128), 0) >= lo - g * 8, blk, oT_s[dst])
            oT_s[dst] = blk

    def f1(t0, c):
        return jnp.dot(xs[pl.ds(t0, TB), :], w1[:, pl.ds(c * FC, FC)], preferred_element_type=f32)

    def mish(hh):
        e = jnp.exp2(jnp.minimum(hh, 30.0))
        n = e * (e + 2.0)
        return ((hh * pl.reciprocal(n + 2.0, approx=True)) * n).astype(bf16)

    def f2(c, act):
        y = jax.lax.dot_general(w2T[:, pl.ds(c * FC * Y, FC * Y)], act, NT_DIMS, preferred_element_type=f32)
        if c == 0:
            yT_s[...] = y
        else:
            yT_s[...] += y

    def combine(i, slot):
        y = yT_s[...]
        g = (y * (1.0 / LOG2E)) * (1.0 / (1.0 + jnp.exp2(-y)))
        out_s[slot] = (xT[:, pl.ds(pl.multiple_of(i * TB, TB), TB)].astype(f32) + sT_s[...] * g).astype(bf16)

    def phase_b(i, c):
        t0 = pl.multiple_of(i * TB, TB)
        slot = i % 2
        nq = TB // 128

        @pl.when(i >= 3)
        def _():
            out_copy(i - 3, 1 - slot).wait()
        pv, hv, av = {}, {}, {}
        un = lambda j: [u for u in range(H * nq) if u * 32 // (H * nq) == j]
        for j in range(NC + 2 - DEF):
            if j == 0 and DEF:
                f2(NC - 1, a_s[...])
            for u in un(j):
                s_s[j % 2, u % nq] = qk_unit(t0, u % nq, u // nq)
            if j < NC:
                hv[j] = f1(t0, j)
            for u in un(j - 1):
                pv[u] = sm_unit(s_s[(j - 1) % 2, u % nq])
            if 0 <= j - 1 < NC:
                av[j - 1] = mish(hv.pop(j - 1))
            if j == 1:
                combine(jnp.maximum(i - 1, 0), 1 - slot)
            for u in un(j - 2):
                pv_unit(t0, u % nq, u // nq, pv.pop(u))
            if 0 <= j - 2 < NC and (j - 2) % Y == Y - 1:
                f2((j - 2) // Y, jnp.concatenate([av.pop(j - 2 - Y + 1 + z) for z in range(Y)], axis=1))
            if j == 35:
                sT_s[...] = jnp.dot(woT[...], oT_s[...].astype(bf16), preferred_element_type=f32)
        if DEF:
            a_s[...] = av.pop(NC - 1)

        @pl.when(i >= 1)
        def _():
            out_copy(i - 1, 1 - slot).start()
        return c

    nb = S // TB
    jax.lax.fori_loop(0, nb, phase_b, 0)
    out_copy(nb - 3, (nb - 3) % 2).wait()
    out_copy(nb - 2, (nb - 2) % 2).wait()
    if DEF:
        f2(NC - 1, a_s[...])
    combine(nb - 1, (nb - 1) % 2)
    out_copy(nb - 1, (nb - 1) % 2).start()
    out_copy(nb - 1, (nb - 1) % 2).wait()


@jax.jit
def pallas_recurrent_scan__sliding_block__dense_activation_mish__prompt_kernel(A_x, A_wqkv, A_wo, B_x, B_w1, B_b1, B_w2):
    del B_x
    any_spec = pl.BlockSpec(memory_space=pl.ANY)
    V = pltpu.VMEM
    oT = pl.pallas_call(
        _kernel,
        out_shape=jax.ShapeDtypeStruct((D, S), bf16),
        in_specs=[any_spec, any_spec, any_spec, any_spec, pl.BlockSpec(memory_space=pltpu.VMEM), any_spec],
        out_specs=any_spec,
        scratch_shapes=[
            V((D, S), bf16), V((D, 2 * D), bf16), V((D, D), bf16), V((D, D), bf16),
            V((DP, F), bf16), V((D, F), bf16),
            V((DP, 2 * DP), bf16), V((D, D), bf16), V((D, D), bf16),
            V((TA, DP), bf16), V((S // 2, DP), i32), V((S, DP), bf16), V((S, DP), bf16), V(((S + W) // 2, DP), i32),
            V((H, (S + W) // 2, 128), i32), V((D, S + W), bf16),
            V((D, TB), f32), V((D, TB), f32), V((D, TB), f32), V((2, TB // 128, 288, 128), f32),
            V((TB, FC), bf16), V((2, D, TB), bf16),
            pltpu.SemaphoreType.DMA((7,)), pltpu.SemaphoreType.DMA((2,)),
        ],
        compiler_params=pltpu.CompilerParams(
            vmem_limit_bytes=100 * 2**20,
            flags={"XLA_TPU_EVENLY_DISTRIBUTE_CRITICAL_NODES": True}),
        name="fused_block",
    )(A_x[0].T, A_wqkv, A_wo, B_w1, B_b1, B_w2.T)
    return oT.T[None]
```

```python
import jax
import jax.numpy as jnp
import jax.experimental.pallas as pl
import jax.experimental.pallas.tpu as pltpu

S, D, F, H, DH, W = 2048, 576, 4608, 32, 18, 256
HPT = 7
NT = 5
DP = NT * 128
TA = 256
TB = 256
FC = 128
FH = F // 2
KH = 256
DHALF = D // 2
NC = FH // FC
NH = 2
ORD = 'qfsmpy'
LOG2E = 1.4426950408889634
L_HI = 1.4453125
ONE2 = 0x3F803F80
NEG2 = 0xCE6ECE6E - (1 << 32)
bf16, f32, i32 = jnp.bfloat16, jnp.float32, jnp.int32
NT_DIMS = (((1,), (1,)), ((), ()))


def mo(x, n):
    return x if isinstance(x, int) else pl.multiple_of(x, n)


def _iota(shape, d):
    return jax.lax.broadcasted_iota(i32, shape, d)


def flag_lane(h):
    return (h % HPT + 4) % HPT * DH


def pack16(x):
    lo = jnp.concatenate([x[r:r + 8] for r in range(0, x.shape[0], 16)], axis=0)
    hi = jnp.concatenate([x[r + 8:r + 16] for r in range(0, x.shape[0], 16)], axis=0)
    return pltpu.pack_elementwise([lo, hi], packed_dtype=bf16).astype(i32)


def lhs_terms(a11, a12, a21, a22):
    return [a11 + a22, a21 + a22, a11, a22, a11 + a12, a21 - a11, a12 - a22]


def rhs_terms(b11, b12, b21, b22):
    return [b11 + b22, b11, b12 - b22, b21 - b11, b22, b11 + b12, b21 + b22]


def out_terms(m, base=None):
    if base is not None:
        return (base[0] + m[0] + m[3] - m[4] + m[6], base[1] + m[2] + m[4], base[2] + m[1] + m[3],
                base[3] + m[0] - m[1] + m[2] + m[5])
    return m[0] + m[3] - m[4] + m[6], m[2] + m[4], m[1] + m[3], m[0] - m[1] + m[2] + m[5]


def _kernel(xT_hbm, wqkv_hbm, wo_hbm, w1_hbm, b1_ref, w2T_hbm, oT_hbm,
            xT, wqk_in, wv, wo, w1, w2T, wqk, wvT, woT, wqc, xp, xs, q_s, k_s, kc_s, vT_s,
            oT_s, yT_s, sT_s, s_s, xl, w1c, w2c, out_s, sem_in, sem_out):
    def x_copy(i):
        lo, n = (0, 2 * TA) if i == 0 else (2 * TA, S - 2 * TA)
        return pltpu.make_async_copy(xT_hbm.at[:, pl.ds(lo, n)], xT.at[:, pl.ds(lo, n)], sem_in.at[i])
    cp_qk = pltpu.make_async_copy(wqkv_hbm.at[:, pl.ds(0, 2 * D)], wqk_in, sem_in.at[2])
    cp_v = pltpu.make_async_copy(wqkv_hbm.at[:, pl.ds(2 * D, D)], wv, sem_in.at[3])
    cp_wo = pltpu.make_async_copy(wo_hbm, wo, sem_in.at[4])
    cp_w1 = pltpu.make_async_copy(w1_hbm, w1.at[pl.ds(0, D), :], sem_in.at[5])
    cp_w2 = pltpu.make_async_copy(w2T_hbm, w2T, sem_in.at[6])
    x_copy(0).start()
    cp_qk.start()

    k_s[pl.ds(0, W // 2), :] = jnp.zeros((W // 2, DP), i32)
    for h in range(H):
        fl = _iota((80, 128), 1) - flag_lane(h)
        kc_s[h, pl.ds(0, 80), :] = jnp.where((fl >= 0) & (fl < 4), NEG2, 0)
    vT_s[:, pl.ds(0, W)] = jnp.zeros((D, W), bf16)
    b1 = jnp.broadcast_to(b1_ref[...].astype(f32).reshape(1, F), (DP - D, F))
    w1[pl.ds(D, DP - D), :] = jnp.where(_iota((DP - D, F), 0) < 2, b1, 0.0).astype(bf16)
    yT_s[...] = jnp.zeros(yT_s.shape, f32)
    sT_s[...] = jnp.zeros(sT_s.shape, f32)
    wqk[...] = jnp.zeros(wqk.shape, bf16)

    def ln(i):
        t0 = mo(i * TA, TA)
        x = xT[:, pl.ds(t0, TA)].astype(f32)
        m = jnp.mean(x, axis=0, keepdims=True)
        xc = x - m
        v = jnp.mean(xc * xc, axis=0, keepdims=True)
        y = xc * jax.lax.rsqrt(v + 1e-5)
        ext = jnp.concatenate([y, jnp.where(_iota((DP - D, TA), 0) == 0, 1.0, 0.0)], axis=0)
        et = ext.T
        xp[pl.ds(mo(t0 // 2, TA // 2), TA // 2), :] = pack16(et)
        ll = _iota((TA, DP), 1)
        el = et * LOG2E
        xs[pl.ds(t0, TA), :] = jnp.where(ll == D, L_HI, jnp.where(ll == D + 1, LOG2E - L_HI, el))[:, 2 * KH:].astype(bf16)
        for n, v in enumerate(lhs_terms(el[:128, :KH], el[:128, KH:2 * KH], el[128:, :KH], el[128:, KH:2 * KH])):
            xl[i, n] = v.astype(bf16)

    def proj(i, extra):
        t0 = mo(i * TA, TA)
        lo, hi = pl.ds(0, DP), pl.ds(DP, DP)
        rhs = [wqc[0], wqk[pl.ds(0, KH), lo], wqc[1], wqc[2], wqk[pl.ds(KH, KH), hi], wqc[3], wqc[4]]
        m = [jnp.dot(xl[i, n], rhs[n], preferred_element_type=f32) for n in range(7)]
        r = jnp.dot(xs[pl.ds(t0, TA), :], wqk[pl.ds(2 * KH, 128), :], preferred_element_type=f32)
        extra()
        q0, k0, q1, k1 = out_terms(m, (r[:128, :DP], r[:128, DP:], r[128:, :DP], r[128:, DP:]))
        for u, (q, k) in enumerate(((q0, k0), (q1, k1))):
            q_s[pl.ds(mo(t0 + 128 * u, 128), 128), :] = (q * (DH ** -0.5 / LOG2E)).astype(bf16)
            k_s[pl.ds(mo((W + t0) // 2 + 64 * u, 64), 64), :] = pltpu.bitcast(k.astype(bf16), i32)

    x_copy(0).wait()
    cp_qk.wait()
    x_copy(1).start()
    cp_v.start()
    cp_wo.start()
    ln(0)
    for part in range(2):
        for t in range(NT):
            n = min(HPT, H - t * HPT) * DH
            wqk[pl.ds(0, D), pl.ds((part * NT + t) * 128, n)] = wqk_in[:, pl.ds(part * D + t * HPT * DH, n)]
    for r in range(0, KH, 16):
        t = rhs_terms(*[wqk[pl.ds(r + o, 16), pl.ds(cc, DP)].astype(f32) for o in (0, KH) for cc in (0, DP)])
        for n, k in enumerate((0, 2, 3, 5, 6)):
            wqc[n, pl.ds(r, 16), :] = t[k].astype(bf16)
    na = S // TA
    nxt = lambda i: jnp.where(i < na, i, 0)
    proj(0, lambda: ln(1))
    x_copy(1).wait()
    cp_v.wait()
    cp_w1.start()
    cp_w2.start()
    wvT[...] = wv[...].astype(f32).T.astype(bf16)

    def v_stair(i):
        t0 = mo(i * TA, TA)
        vT_s[:, pl.ds(W + t0, TA)] = jax.lax.dot_general(wvT[...], pltpu.bitcast(xp[pl.ds(mo(t0 // 2, TA // 2), TA // 2), pl.ds(0, D)], bf16), NT_DIMS, preferred_element_type=f32).astype(bf16)
        r0 = mo(t0 // 2 + 80, 16)
        lane = _iota((TA // 2, 128), 1)
        for t in range(NT):
            rolled = {}
            for j in range(min(HPT, H - t * HPT)):
                x = 0
                for g in range(4):
                    sl = (j + g) % HPT
                    if sl - j not in rolled:
                        src = k_s[pl.ds(r0 + 16 * g, TA // 2), pl.ds(t * 128, 128)]
                        rolled[sl - j] = src if g == 0 else pltpu.roll(src, (DH * (sl - j)) % 128, 1)
                    x = jnp.where((lane >= sl * DH) & (lane < (sl + 1) * DH), rolled[sl - j], x)
                kc_s[t * HPT + j, pl.ds(r0, TA // 2), :] = x

    def weight_terms(c, carry):
        lo, hi = pl.ds(mo(c * FC, FC), FC), pl.ds(mo(FH + c * FC, FC), FC)
        for r in range(0, KH, 32):
            t = rhs_terms(*[w1[pl.ds(r + o, 32), cc].astype(f32) for o in (0, KH) for cc in (lo, hi)])
            for n, k in enumerate((0, 2, 3, 5, 6)):
                w1c[n, pl.ds(r, 32), lo] = t[k].astype(bf16)
        for r in range(0, DHALF, 32):
            t = lhs_terms(*[w2T[pl.ds(r + o, 32), cc].astype(f32) for o in (0, DHALF) for cc in (lo, hi)])
            for n, k in enumerate((0, 1, 4, 5, 6)):
                w2c[n, pl.ds(r, 32), lo] = t[k].astype(bf16)
        return carry

    def phase_a(i, c):
        v_stair(i - 1)
        proj(i, lambda: ln(nxt(i + 1)))
        return c
    NW = 2
    jax.lax.fori_loop(1, na - NW, phase_a, 0)
    cp_w1.wait()
    cp_w2.wait()

    def phase_a_w(i, c):
        for k in range(NC // NW):
            weight_terms((i - (na - NW)) * (NC // NW) + k, 0)
        return phase_a(i, c)
    jax.lax.fori_loop(na - NW, na, phase_a_w, 0)
    cp_wo.wait()
    v_stair(na - 1)
    for h in range(H):
        fl = _iota((48, 128), 1) - flag_lane(h)
        pad = (fl >= 0) & (fl < 4) & (2 * (_iota((48, 128), 0) + 80) + 32 * fl < W)
        kc_s[h, pl.ds(80, 48), :] = jnp.where(pad, NEG2, kc_s[h, pl.ds(80, 48), :])
    woT[...] = wo[...].astype(f32).T.astype(bf16)


    def out_copy(i, slot):
        return pltpu.make_async_copy(out_s.at[slot], oT_hbm.at[:, pl.ds(i * TB, TB)], sem_out.at[slot])

    def qk_unit(t0, qb, h):
        t, j = divmod(h, HPT)
        ln_ = _iota((16, 128), 1)
        qt = pltpu.bitcast(q_s[pl.ds(t0 + qb * 128, 128), pl.ds(t * 128, 128)], i32)
        parts = []
        for g in range(4):
            x = qt[16 * g:16 * g + 16]
            sl = (j + g) % HPT
            if g:
                x = pltpu.roll(x, (DH * (sl - j)) % 128, 1)
            parts.append(jnp.where((ln_ >= sl * DH) & (ln_ < (sl + 1) * DH), x, jnp.where(ln_ == flag_lane(h) + g, ONE2, 0)))
        qm = pltpu.bitcast(jnp.concatenate(parts, axis=0), bf16)
        kt = pltpu.bitcast(kc_s[h, pl.ds(pl.multiple_of((t0 + qb * 128) // 2, 64), 144), :], bf16)
        return jax.lax.dot_general(kt, qm, NT_DIMS, preferred_element_type=f32)

    def sm_unit(s):
        ln_ = _iota((32, 128), 1)
        up = _iota((32, 128), 0) > (ln_ & 31)
        s0 = jnp.where(up, s[0:32], s[256:288])
        s1 = s[32:256]
        mx = jnp.maximum(jnp.max(s0, axis=0, keepdims=True), jnp.max(s1, axis=0, keepdims=True))
        p0 = jnp.exp2(s0 - mx)
        p1 = jnp.exp2(s1 - mx)
        c = [jnp.where(up, p0, 0.0)] + [p1[32 * n:32 * n + 32] for n in range(7)] + [jnp.where(up, 0.0, p0)]
        c = [pack16(x) for x in c]
        l16 = _iota((16, 128), 1)
        odd = (l16 & 32) != 0
        hi = l16 >= 64
        c = [jnp.where(odd, c[n - 1] if n >= 1 else 0, c[n] if n < 9 else 0) for n in range(10)]
        c = [jnp.where(hi, c[n - 2] if n >= 2 else 0, c[n] if n < 10 else 0) for n in range(12)]
        return pltpu.bitcast(jnp.concatenate(c, axis=0), bf16)

    def pv_unit(t0, qb, h, p):
        a = (h * DH) // 16 * 16
        vt = vT_s[pl.ds(a, 32), pl.ds(t0 + qb * 128, 384)]
        lo, hi = h * DH, (h + 1) * DH
        r = 0 if lo > a else 30
        vt = pltpu.bitcast(jnp.where(_iota((16, 384), 0) == r // 2, ONE2, pltpu.bitcast(vt, i32)), bf16)
        o = jnp.dot(vt, p, preferred_element_type=f32)
        o = o * (1.0 / o[r:r + 1])
        for g in range(lo // 8, (hi + 7) // 8):
            blk = o[g * 8 - a:g * 8 - a + 8]
            dst = (pl.ds(g * 8, 8), pl.ds(qb * 128, 128))
            if g * 8 < lo:
                blk = jnp.where(_iota((8, 128), 0) >= lo - g * 8, blk, oT_s[dst])
            oT_s[dst] = blk

    def f1(i, t0, c):
        lo, hi = pl.ds(c * FC, FC), pl.ds(FH + c * FC, FC)
        rhs = [w1c.at[0, :, lo], w1.at[pl.ds(0, KH), lo], w1c.at[1, :, lo], w1c.at[2, :, lo],
               w1.at[pl.ds(KH, KH), hi], w1c.at[3, :, lo], w1c.at[4, :, lo]]
        mm = lambda a, b: (lambda: jnp.dot(a[...], b[...], preferred_element_type=f32))
        xr = xs.at[pl.ds(t0, TB), :]
        return [mm(xl.at[i, n], rhs[n]) for n in range(7)] + [mm(xr, w1.at[pl.ds(2 * KH, 128), cc]) for cc in (lo, hi)]

    def mish(hh):
        e = jnp.exp2(jnp.minimum(hh, 30.0))
        n = e * (e + 2.0)
        return (hh * pl.reciprocal(n + 2.0, approx=True)) * n

    def f2(c, acts, which):
        lo, hi = pl.ds(c * FC, FC), pl.ds(FH + c * FC, FC)
        lhs = [w2c[0, :, lo], w2c[1, :, lo], w2T[pl.ds(0, DHALF), lo], w2T[pl.ds(DHALF, DHALF), hi],
               w2c[2, :, lo], w2c[3, :, lo], w2c[4, :, lo]]
        for n in which:
            y = jax.lax.dot_general(lhs[n], acts[n], NT_DIMS, preferred_element_type=f32)
            if c == 0:
                yT_s[n] = y
            else:
                yT_s[n] += y

    def combine(i, slot):
        c11, c12, c21, c22 = out_terms([yT_s[n] for n in range(7)])
        y = jnp.concatenate([jnp.concatenate([c11, c12], axis=1), jnp.concatenate([c21, c22], axis=1)], axis=0)
        g = (y * (1.0 / LOG2E)) * (1.0 / (1.0 + jnp.exp2(-y)))
        out_s[slot] = (xT[:, pl.ds(pl.multiple_of(i * TB, TB), TB)].astype(f32) + sT_s[...] * g).astype(bf16)

    def phase_b(i, c):
        t0 = pl.multiple_of(i * TB, TB)
        slot = i % 2
        nq = TB // 128

        @pl.when(i >= 3)
        def _():
            out_copy(i - 3, 1 - slot).wait()
        pv, hv, av = {}, {}, {}
        un = lambda j: [u for u in range(H * nq) if u * 16 // (H * nq) == j]
        for j in range(NC + 2):
            for half in range(NH):
                part = lambda xs_, h=half: xs_[len(xs_) * h // NH:len(xs_) * (h + 1) // NH]
                for ch in ORD:
                    if ch == 'q':
                        for u in part(un(j)):
                            s_s[j % 2, u % 4] = qk_unit(t0, u % nq, u // nq)
                    if ch == 'f' and j < NC:
                        hv.setdefault(j, []).extend(f() for f in part(f1(i, t0, j)))
                    if ch == 's':
                        for u in part(un(j - 1)):
                            pv[u] = sm_unit(s_s[(j - 1) % 2, u % 4])
                    if ch == 'm' and 0 <= j - 1 < NC:
                        m = hv[j - 1]
                        hh = out_terms(m, (m[7][:128], m[8][:128], m[7][128:], m[8][128:]))
                        hh = (hh[0], hh[2], hh[1], hh[3])
                        av.setdefault(j - 1, []).extend(mish(v) for v in part(hh))
                    if ch == 'p':
                        for u in part(un(j - 2)):
                            pv_unit(t0, u % nq, u // nq, pv.pop(u))
                    if ch == 'y' and 0 <= j - 2 < NC:
                        f2(j - 2, av[j - 2], part(range(7)))
            if 0 <= j - 1 < NC:
                av[j - 1] = [v.astype(bf16) for v in rhs_terms(*av[j - 1])]
            if j == 1:
                combine(jnp.maximum(i - 1, 0), 1 - slot)
            if j == 17:
                sT_s[...] = jnp.dot(woT[...], oT_s[...].astype(bf16), preferred_element_type=f32)

        @pl.when(i >= 1)
        def _():
            out_copy(i - 1, 1 - slot).start()
        return c

    nb = S // TB
    jax.lax.fori_loop(0, nb, phase_b, 0)
    out_copy(nb - 3, (nb - 3) % 2).wait()
    out_copy(nb - 2, (nb - 2) % 2).wait()
    combine(nb - 1, (nb - 1) % 2)
    out_copy(nb - 1, (nb - 1) % 2).start()
    out_copy(nb - 1, (nb - 1) % 2).wait()


@jax.jit
def pallas_recurrent_scan__sliding_block__dense_activation_mish__prompt_kernel(A_x, A_wqkv, A_wo, B_x, B_w1, B_b1, B_w2):
    del B_x
    any_spec = pl.BlockSpec(memory_space=pl.ANY)
    V = pltpu.VMEM
    oT = pl.pallas_call(
        _kernel,
        out_shape=jax.ShapeDtypeStruct((D, S), bf16),
        in_specs=[any_spec, any_spec, any_spec, any_spec, pl.BlockSpec(memory_space=pltpu.VMEM), any_spec],
        out_specs=any_spec,
        scratch_shapes=[
            V((D, S), bf16), V((D, 2 * D), bf16), V((D, D), bf16), V((D, D), bf16),
            V((DP, F), bf16), V((D, F), bf16),
            V((DP, 2 * DP), bf16), V((D, D), bf16), V((D, D), bf16),
            V((5, KH, DP), bf16), V((S // 2, DP), i32), V((S, 128), bf16), V((S, DP), bf16), V(((S + W) // 2, DP), i32),
            V((H, (S + W) // 2, 128), i32), V((D, S + W), bf16),
            V((D, TB), f32), V((7, DHALF, 128), f32), V((D, TB), f32), V((2, 4, 288, 128), f32),
            V((S // TA, 7, 128, KH), bf16), V((5, KH, FH), bf16), V((5, DHALF, FH), bf16), V((2, D, TB), bf16),
            pltpu.SemaphoreType.DMA((7,)), pltpu.SemaphoreType.DMA((2,)),
        ],
        compiler_params=pltpu.CompilerParams(
            vmem_limit_bytes=100 * 2**20,
            flags={"XLA_TPU_EVENLY_DISTRIBUTE_CRITICAL_NODES": True}),
        name="fused_block",
    )(A_x[0].T, A_wqkv, A_wo, B_w1, B_b1, B_w2.T)
    return oT.T[None]
```

```python
import jax
import jax.numpy as jnp
import jax.experimental.pallas as pl
import jax.experimental.pallas.tpu as pltpu

S, D, F, H, DH, W = 2048, 576, 4608, 32, 18, 256
HPT = 7
NT = 5
DP = NT * 128
TB = 256
NB = S // TB
FC = 128
FH, KH, DHALF = F // 2, 256, D // 2
NC = FH // FC
LOG2E = 1.4426950408889634
L_HI = 1.4453125
ONE2 = 0x3F803F80
NEG2 = 0xCE6ECE6E - (1 << 32)
bf16, f32, i32 = jnp.bfloat16, jnp.float32, jnp.int32
NT_DIMS = (((1,), (1,)), ((), ()))


def mo(x, n):
    return x if isinstance(x, int) else pl.multiple_of(x, n)


def _iota(shape, d):
    return jax.lax.broadcasted_iota(i32, shape, d)


def flag_lane(h):
    return (h % HPT + 4) % HPT * DH


def words(x):
    return pltpu.bitcast(x.astype(bf16), i32)


def halves(x):
    return pltpu.bitcast(x, bf16)


def pack16(x):
    lo = jnp.concatenate([x[r:r + 8] for r in range(0, x.shape[0], 16)], axis=0)
    hi = jnp.concatenate([x[r + 8:r + 16] for r in range(0, x.shape[0], 16)], axis=0)
    return pltpu.pack_elementwise([lo, hi], packed_dtype=bf16).astype(i32)


def lhs_terms(a11, a12, a21, a22):
    return [a11 + a22, a21 + a22, a11, a22, a11 + a12, a21 - a11, a12 - a22]


def rhs_terms(b11, b12, b21, b22):
    return [b11 + b22, b11, b12 - b22, b21 - b11, b22, b11 + b12, b21 + b22]


def word_terms(fn, blocks):
    lo = [pltpu.bitcast(b << 16, f32) for b in blocks]
    hi = [pltpu.bitcast(b & -65536, f32) for b in blocks]
    out = []
    for a, b in zip(fn(*lo), fn(*hi)):
        same = [blk for blk, v in zip(blocks, lo) if v is a]
        out.append(same[0] if same else pltpu.pack_elementwise([a, b], packed_dtype=bf16).astype(i32))
    return out


def out_terms(m, base):
    return (base[0] + m[0] + m[3] - m[4] + m[6], base[1] + m[2] + m[4], base[2] + m[1] + m[3],
            base[3] + m[0] - m[1] + m[2] + m[5])


def dot(a, b):
    return jnp.dot(a, b, preferred_element_type=f32)


def dot_nt(a, b):
    return jax.lax.dot_general(a, b, NT_DIMS, preferred_element_type=f32)


def _kernel(xT_hbm, wqkv_hbm, wo_hbm, w1_hbm, b1_ref, w2T_hbm, oT_hbm,
            xT, wqk_in, wv, wo, w1, w2T, wqk, wvT, woT, w1c, w1r, w2c,
            xn, xp, xs, xl, q_s, k_s, kc_s, vT_s, oT_s, yT_s, sT_s, s_s, out_s, sem_in, sem_out):
    def x_copy(i):
        lo, n = (0, 2 * TB) if i == 0 else (2 * TB, S - 2 * TB)
        return pltpu.make_async_copy(xT_hbm.at[:, pl.ds(lo, n)], xT.at[:, pl.ds(lo, n)], sem_in.at[i])
    cp_qk = pltpu.make_async_copy(wqkv_hbm.at[:, pl.ds(0, 2 * D)], wqk_in, sem_in.at[2])
    cp_v = pltpu.make_async_copy(wqkv_hbm.at[:, pl.ds(2 * D, D)], wv, sem_in.at[3])
    cp_wo = pltpu.make_async_copy(wo_hbm, wo, sem_in.at[4])
    cp_w1 = pltpu.make_async_copy(w1_hbm, w1, sem_in.at[5])
    cp_w2 = pltpu.make_async_copy(w2T_hbm, w2T, sem_in.at[6])
    x_copy(0).start()
    cp_qk.start()

    k_s[pl.ds(0, W // 2), :] = jnp.zeros((W // 2, DP), i32)
    for h in range(H):
        fl = _iota((80, 128), 1) - flag_lane(h)
        kc_s[h, pl.ds(0, 80), :] = jnp.where((fl >= 0) & (fl < 4), NEG2, 0)
    vT_s[:, pl.ds(0, W)] = jnp.zeros((D // 2, W), i32)
    b1 = jnp.broadcast_to(b1_ref[...].astype(f32).reshape(1, F), (DP - D, F))
    w1r[pl.ds(32, 32), :] = words(jnp.where(_iota((DP - D, F), 0) < 2, b1, 0.0))
    yT_s[...] = jnp.zeros(yT_s.shape, f32)
    sT_s[...] = jnp.zeros(sT_s.shape, f32)
    wqk[...] = jnp.zeros(wqk.shape, i32)

    def ln(i):
        t0 = mo(i * TB, TB)
        r0 = mo(i * (TB // 2), TB // 2)
        x = xT[:, pl.ds(t0, TB)].astype(f32)
        xc = x - jnp.mean(x, axis=0, keepdims=True)
        y = xc * jax.lax.rsqrt(jnp.mean(xc * xc, axis=0, keepdims=True) + 1e-5)
        et = jnp.concatenate([y, jnp.zeros((DP - D, TB), f32)], axis=0).T
        xn[...] = words(et)
        xp[pl.ds(r0, TB // 2), :] = pack16(et)
        el = et * LOG2E
        ll = _iota((TB, 128), 1) + 2 * KH
        xs[pl.ds(r0, TB // 2), :] = words(jnp.where(ll == D, L_HI, jnp.where(ll == D + 1, LOG2E - L_HI, el[:, 2 * KH:])))
        for n, v in enumerate(lhs_terms(el[:128, :KH], el[:128, KH:2 * KH], el[128:, :KH], el[128:, KH:2 * KH])):
            xl[i, n] = words(v)

    def proj(i, extra):
        r0 = mo(i * (TB // 2), TB // 2)
        qk = dot(halves(xn[...]), halves(wqk[...]))
        extra()
        q_s[pl.ds(r0, TB // 2), :] = words(qk[:, :DP] * (DH ** -0.5 * LOG2E))
        k_s[pl.ds(mo(W // 2 + r0, TB // 2), TB // 2), :] = words(qk[:, DP:])

    def v_stair(i):
        r0 = mo(i * (TB // 2), TB // 2)
        vT_s[:, pl.ds(mo(W + i * TB, TB), TB)] = words(dot_nt(halves(wvT[...]), halves(xp[pl.ds(r0, TB // 2), pl.ds(0, D)])))
        r0 = mo(r0 + 80, 16)
        lane = _iota((TB // 2, 128), 1)
        for t in range(NT):
            rolled = {}
            for j in range(min(HPT, H - t * HPT)):
                x = 0
                for g in range(4):
                    sl = (j + g) % HPT
                    if sl - j not in rolled:
                        src = k_s[pl.ds(r0 + 16 * g, TB // 2), pl.ds(t * 128, 128)]
                        rolled[sl - j] = src if g == 0 else pltpu.roll(src, (DH * (sl - j)) % 128, 1)
                    x = jnp.where((lane >= sl * DH) & (lane < (sl + 1) * DH), rolled[sl - j], x)
                kc_s[t * HPT + j, pl.ds(r0, TB // 2), :] = x

    def weight_terms(c):
        lo, hi = pl.ds(mo(c * FC, FC), FC), pl.ds(mo(FH + c * FC, FC), FC)
        for r in range(0, KH, 32):
            t = word_terms(rhs_terms, [words(w1[pl.ds(r + o, 32), cc]) for o in (0, KH) for cc in (lo, hi)])
            for n in range(7):
                w1c[n, pl.ds(r // 2, 16), lo] = t[n]
        for cc in (lo, hi):
            w1r[pl.ds(0, 32), cc] = words(w1[pl.ds(2 * KH, D - 2 * KH), cc])
        for r in range(0, DHALF, 32):
            t = word_terms(lhs_terms, [words(w2T[pl.ds(r + o, 32), cc]) for o in (0, DHALF) for cc in (lo, hi)])
            for n in range(7):
                w2c[n, pl.ds(r // 2, 16), lo] = t[n]

    x_copy(0).wait()
    cp_qk.wait()
    x_copy(1).start()
    cp_v.start()
    cp_wo.start()
    ln(0)
    wq_words = words(wqk_in[...])
    for part in range(2):
        for t in range(NT):
            n = min(HPT, H - t * HPT) * DH
            src = part * D + t * HPT * DH
            wqk[pl.ds(0, D // 2), pl.ds((part * NT + t) * 128, n)] = wq_words[:, src:src + n]
    proj(0, lambda: ln(1))
    x_copy(1).wait()
    cp_v.wait()
    cp_w1.start()
    cp_w2.start()
    wvT[...] = words(wv[...].astype(f32).T)

    def phase_a(i, c):
        v_stair(i - 1)
        proj(i, lambda: ln(jnp.where(i + 1 < NB, i + 1, 0)))
        return c

    NW = 2

    def phase_a_w(i, c):
        for k in range(NC // NW):
            weight_terms((i - (NB - NW)) * (NC // NW) + k)
        return phase_a(i, c)

    jax.lax.fori_loop(1, NB - NW, phase_a, 0)
    cp_w1.wait()
    cp_w2.wait()
    jax.lax.fori_loop(NB - NW, NB, phase_a_w, 0)
    cp_wo.wait()
    v_stair(NB - 1)
    for h in range(H):
        fl = _iota((48, 128), 1) - flag_lane(h)
        pad = (fl >= 0) & (fl < 4) & (2 * (_iota((48, 128), 0) + 80) + 32 * fl < W)
        kc_s[h, pl.ds(80, 48), :] = jnp.where(pad, NEG2, kc_s[h, pl.ds(80, 48), :])
    woT[...] = words(wo[...].astype(f32).T)

    def out_copy(i, slot):
        return pltpu.make_async_copy(out_s.at[slot], oT_hbm.at[:, pl.ds(i * TB, TB)], sem_out.at[slot])

    def qk_unit(i, qb, h):
        t, j = divmod(h, HPT)
        r0 = mo(i * (TB // 2) + qb * 64, 64)
        lane = _iota((16, 128), 1)
        parts = []
        for g in range(4):
            x = q_s[pl.ds(r0 + 16 * g, 16), pl.ds(t * 128, 128)]
            sl = (j + g) % HPT
            if g:
                x = pltpu.roll(x, (DH * (sl - j)) % 128, 1)
            parts.append(jnp.where((lane >= sl * DH) & (lane < (sl + 1) * DH), x, jnp.where(lane == flag_lane(h) + g, ONE2, 0)))
        return dot_nt(halves(kc_s[h, pl.ds(r0, 144), :]), halves(jnp.concatenate(parts, axis=0)))

    def sm_unit(s):
        up = _iota((32, 128), 0) > (_iota((32, 128), 1) & 31)
        s0 = jnp.where(up, s[0:32], s[256:288])
        s1 = s[32:256]
        mx = jnp.maximum(jnp.max(s0, axis=0, keepdims=True), jnp.max(s1, axis=0, keepdims=True))
        p0 = jnp.exp2(s0 - mx)
        p1 = jnp.exp2(s1 - mx)
        c = [jnp.where(up, p0, 0.0)] + [p1[32 * n:32 * n + 32] for n in range(7)] + [jnp.where(up, 0.0, p0)]
        c = [pack16(x) for x in c]
        lane = _iota((16, 128), 1)
        odd, hi = (lane & 32) != 0, lane >= 64
        c = [jnp.where(odd, c[n - 1] if n >= 1 else 0, c[n] if n < 9 else 0) for n in range(10)]
        c = [jnp.where(hi, c[n - 2] if n >= 2 else 0, c[n] if n < 10 else 0) for n in range(12)]
        return halves(jnp.concatenate(c, axis=0))

    def pv_unit(i, qb, h, p):
        lo, hi = h * DH, (h + 1) * DH
        a = lo // 16 * 16
        r = 0 if lo > a else 30
        vt = vT_s[pl.ds(a // 2, 16), pl.ds(mo(i * TB + qb * 128, 128), 384)]
        o = dot(halves(jnp.where(_iota((16, 384), 0) == r // 2, ONE2, vt)), p)
        o = o * (1.0 / o[r:r + 1])
        for g in range(lo // 8, (hi + 7) // 8):
            blk = o[g * 8 - a:g * 8 - a + 8]
            dst = (pl.ds(g * 8, 8), pl.ds(qb * 128, 128))
            if g * 8 < lo:
                blk = jnp.where(_iota((8, 128), 0) >= lo - g * 8, blk, oT_s[dst])
            oT_s[dst] = blk

    def f1(i, c, n):
        if n < 7:
            return dot(halves(xl[i, n]), halves(w1c[n, :, pl.ds(c * FC, FC)]))
        return dot(halves(xs[pl.ds(mo(i * (TB // 2), TB // 2), TB // 2), :]), halves(w1r[:, pl.ds((n - 7) * FH + c * FC, FC)]))

    def mish(hh):
        e = jnp.exp2(jnp.minimum(hh, 30.0))
        n = e * (e + 2.0)
        return (hh * pl.reciprocal(n + 2.0, approx=True)) * n

    def f2(c, n, act):
        y = dot_nt(halves(w2c[n, :, pl.ds(c * FC, FC)]), act)
        if c == 0:
            yT_s[n] = y
        else:
            yT_s[n] += y

    def combine(i, slot):
        m = [yT_s[n] for n in range(7)]
        c11, c12, c21, c22 = m[0] + m[3] - m[4] + m[6], m[2] + m[4], m[1] + m[3], m[0] - m[1] + m[2] + m[5]
        y = jnp.concatenate([jnp.concatenate([c11, c12], axis=1), jnp.concatenate([c21, c22], axis=1)], axis=0)
        g = (y * (1.0 / LOG2E)) * (1.0 / (1.0 + jnp.exp2(-y)))
        out_s[slot] = (xT[:, pl.ds(mo(i * TB, TB), TB)].astype(f32) + sT_s[...] * g).astype(bf16)

    NH, ORD, SP = 4, 'qfsmpy', 16

    def phase_b(i, c):
        slot = i % 2

        @pl.when(i >= 3)
        def _():
            out_copy(i - 3, 1 - slot).wait()
        pv, hv, av = {}, {}, {}
        un = lambda j: [u for u in range(2 * H) if u * SP // (2 * H) == j]
        for j in range(NC + 2):
            for half in range(NH):
                part = lambda v: v[len(v) * half // NH:len(v) * (half + 1) // NH]
                for ch in ORD:
                    if ch == 'q':
                        for u in part(un(j)):
                            s_s[j % 2, u % 4] = qk_unit(i, u % 2, u // 2)
                    if ch == 'f' and j < NC:
                        hv.setdefault(j, []).extend([f1(i, j, n) for n in part(range(9))])
                    if ch == 's':
                        for u in part(un(j - 1)):
                            pv[u] = sm_unit(s_s[(j - 1) % 2, u % 4])
                    if ch == 'm' and 0 <= j - 1 < NC:
                        m = hv[j - 1]
                        hh = out_terms(m, (m[7][:128], m[8][:128], m[7][128:], m[8][128:]))
                        hh = (hh[0], hh[2], hh[1], hh[3])
                        av.setdefault(j - 1, []).extend([mish(v) for v in part(hh)])
                    if ch == 'p':
                        for u in part(un(j - 2)):
                            pv_unit(i, u % 2, u // 2, pv.pop(u))
                    if ch == 'y' and 0 <= j - 2 < NC:
                        for n in part(range(7)):
                            f2(j - 2, n, av[j - 2][n])
            if 0 <= j - 1 < NC:
                av[j - 1] = [v.astype(bf16) for v in rhs_terms(*av[j - 1])]
            if j == 1:
                combine(jnp.maximum(i - 1, 0), 1 - slot)
            if j == 19:
                sT_s[...] = dot(halves(woT[...]), oT_s[...].astype(bf16))

        @pl.when(i >= 1)
        def _():
            out_copy(i - 1, 1 - slot).start()
        return c

    jax.lax.fori_loop(0, NB, phase_b, 0)
    out_copy(NB - 3, (NB - 3) % 2).wait()
    out_copy(NB - 2, (NB - 2) % 2).wait()
    combine(NB - 1, (NB - 1) % 2)
    out_copy(NB - 1, (NB - 1) % 2).start()
    out_copy(NB - 1, (NB - 1) % 2).wait()


@jax.jit
def pallas_recurrent_scan__sliding_block__dense_activation_mish__prompt_kernel(A_x, A_wqkv, A_wo, B_x, B_w1, B_b1, B_w2):
    del B_x
    any_spec = pl.BlockSpec(memory_space=pl.ANY)
    V = pltpu.VMEM
    oT = pl.pallas_call(
        _kernel,
        out_shape=jax.ShapeDtypeStruct((D, S), bf16),
        in_specs=[any_spec, any_spec, any_spec, any_spec, pl.BlockSpec(memory_space=pltpu.VMEM), any_spec],
        out_specs=any_spec,
        scratch_shapes=[
            V((D, S), bf16), V((D, 2 * D), bf16), V((D, D), bf16), V((D, D), bf16), V((D, F), bf16), V((D, F), bf16),
            V((DP // 2, 2 * DP), i32), V((D // 2, D), i32), V((D // 2, D), i32),
            V((7, KH // 2, FH), i32), V((64, F), i32), V((7, DHALF // 2, FH), i32),
            V((TB // 2, DP), i32), V((S // 2, DP), i32), V((S // 2, 128), i32), V((NB, 7, 64, KH), i32),
            V((S // 2, DP), i32), V(((S + W) // 2, DP), i32), V((H, (S + W) // 2, 128), i32), V((D // 2, S + W), i32),
            V((D, TB), f32), V((7, DHALF, 128), f32), V((D, TB), f32), V((2, 4, 288, 128), f32), V((2, D, TB), bf16),
            pltpu.SemaphoreType.DMA((7,)), pltpu.SemaphoreType.DMA((2,)),
        ],
        compiler_params=pltpu.CompilerParams(
            vmem_limit_bytes=110 * 2**20,
            flags={"XLA_TPU_EVENLY_DISTRIBUTE_CRITICAL_NODES": True}),
        name="fused_block",
    )(A_x[0].T, A_wqkv, A_wo, B_w1, B_b1, B_w2.T)
    return oT.T[None]
```
